```python
import os as _os
_os.environ.setdefault("JAX_PLATFORMS", "cpu")
import jax
import jax.numpy as jnp

def _softmax(x, axis=-1):
    return jax.nn.softmax(x, axis=axis)
def _gelu(x):
    return jax.nn.gelu(x, approximate=True)
def _silu(x):
    return jax.nn.silu(x)
def _sigmoid(x):
    return jax.nn.sigmoid(x)
def _layernorm(x, axis=-1, eps=1e-5):
    m = jnp.mean(x, axis=axis, keepdims=True)
    v = jnp.var(x, axis=axis, keepdims=True)
    return (x - m) / jnp.sqrt(v + eps)
def _scatter_add(tgt, idx, src, axis=0):
    return tgt.at[idx].add(src)
def _segment_sum(src, seg, n):
    return jax.ops.segment_sum(src, seg, n)
class _Rng:
    def __init__(self, key):
        self._k = key
    def _next(self):
        self._k, sub = jax.random.split(self._k)
        return sub
    def normal(self, shape):
        return jax.random.normal(self._next(), shape, dtype=jnp.bfloat16)
    def randint(self, lo, hi, shape):
        return jax.random.randint(self._next(), shape, lo, hi, dtype=jnp.int32)
    def uniform(self, shape, lo=0.0, hi=1.0):
        return jax.random.uniform(self._next(), shape, jnp.bfloat16, lo, hi)
    def permutation(self, n):
        return jax.random.permutation(self._next(), n)


kernel_name = 'recurrent_scan__ssm_conv_s5__mixer_s_mlp__prompt'

def setup_inputs():
    _rng = _Rng(jax.random.key(int.from_bytes(__import__("os").urandom(4), "little")))
    _w = (lambda a: (lambda t: t.astype(jnp.bfloat16) if jnp.issubdtype(t.dtype, jnp.floating) else t)(jnp.asarray(a)))
    def _A_setup():
        B, S, D = 1, 2048, 640
        P = D
        Lambda_re = -0.5 * jnp.exp((lambda *s: _rng.normal(s) * 0.8)(P))
        Lambda_im = (lambda *s: _rng.normal(s) * 0.8)(P) * 1.0
        B_re = (lambda *s: _rng.normal(s) * 0.8)(P, D) * (D ** -0.5)
        B_im = (lambda *s: _rng.normal(s) * 0.8)(P, D) * (D ** -0.5)
        C_re = (lambda *s: _rng.normal(s) * 0.8)(D, P) * (P ** -0.5)
        C_im = (lambda *s: _rng.normal(s) * 0.8)(D, P) * (P ** -0.5)
        log_dt = (lambda *s: _rng.normal(s) * 0.8)(P) * 0.3 - 2.0
        Dskip = (lambda *s: _rng.normal(s) * 0.8)(D)
        return {
            "x": _w((lambda *s: _rng.normal(s) * 0.05)(B, S, D)),
            "Lambda_re": _w(Lambda_re),
            "Lambda_im": _w(Lambda_im),
            "B_re": _w(B_re),
            "B_im": _w(B_im),
            "C_re": _w(C_re),
            "C_im": _w(C_im),
            "log_dt": _w(log_dt),
            "Dskip": _w(Dskip),
        }
    _A_in = _A_setup()

    def _B_setup():
        B, S, D, F = 1, 2048, 640, 1536
        return {
            "x":  _w((lambda *s: _rng.normal(s) * 0.05)(B, S, D)),
            "w1": _w((lambda *s: _rng.normal(s) * 0.8)(D, D) * (D ** -0.5)),
            "w2": _w((lambda *s: _rng.normal(s) * 0.8)(D, D) * (D ** -0.5)),
            "w3": _w((lambda *s: _rng.normal(s) * 0.8)(D, F) * (D ** -0.5)),
            "w4": _w((lambda *s: _rng.normal(s) * 0.8)(F, D) * (F ** -0.5)),
        }
    _B_in = _B_setup()

    return {
        "A_x": _A_in["x"],
        "A_Lambda_re": _A_in["Lambda_re"],
        "A_Lambda_im": _A_in["Lambda_im"],
        "A_B_re": _A_in["B_re"],
        "A_B_im": _A_in["B_im"],
        "A_C_re": _A_in["C_re"],
        "A_C_im": _A_in["C_im"],
        "A_log_dt": _A_in["log_dt"],
        "A_Dskip": _A_in["Dskip"],
        "B_x": _B_in["x"],
        "B_w1": _B_in["w1"],
        "B_w2": _B_in["w2"],
        "B_w3": _B_in["w3"],
        "B_w4": _B_in["w4"],
    }

def reference(A_x, A_Lambda_re, A_Lambda_im, A_B_re, A_B_im, A_C_re, A_C_im, A_log_dt, A_Dskip, B_x, B_w1, B_w2, B_w3, B_w4):
    def _A_ref(x, Lambda_re, Lambda_im, B_re, B_im, C_re, C_im, log_dt, Dskip):
        Bsz, L, H = x.shape
        Lam = Lambda_re + 1j * Lambda_im
        Bmat = B_re + 1j * B_im
        Cmat = C_re + 1j * C_im
        dt = jnp.exp(log_dt)
        Lam_bar = jnp.exp(dt * Lam)
        B_bar = ((Lam_bar - 1.0) / Lam)[:, None] * Bmat
        Bu = jnp.einsum("bld,pd->blp", x + 0j, B_bar)
        h = jnp.zeros_like(Bu[:, 0, :])
        hs = []
        for t in range(L):
            h = Lam_bar[None, :] * h + Bu[:, t, :]
            hs.append(h)
        hseq = jnp.stack(hs, 1)
        y = 2.0 * jnp.einsum("blp,dp->bld", hseq, Cmat).real + x * Dskip[None, None, :]
        return y

    def _B_ref(x, w1, w2, w3, w4):
        B, S, D = x.shape
        h = _gelu(_layernorm(x, axis=-1) @ w1)
        c = D // 4
        g0 = jnp.pad(h[:, :, 0*c:1*c], ((0, 0), (1, 0), (0, 0)))[:, :S, :]
        g1 = jnp.pad(h[:, :, 1*c:2*c], ((0, 0), (0, 1), (0, 0)))[:, 1:, :]
        g2 = jnp.pad(h[:, :, 2*c:3*c], ((0, 0), (2, 0), (0, 0)))[:, :S, :]
        g3 = jnp.pad(h[:, :, 3*c:   ], ((0, 0), (0, 2), (0, 0)))[:, 2:, :]
        hs = jnp.concatenate([g0, g1, g2, g3], axis=-1) @ w2
        x1 = x + hs
        h2 = _gelu(_layernorm(x1, axis=-1) @ w3) @ w4
        return x1 + h2

    x = A_x
    xn = _layernorm(x, axis=-1)
    s = _A_ref(xn, A_Lambda_re, A_Lambda_im, A_B_re, A_B_im, A_C_re, A_C_im, A_log_dt, A_Dskip)
    g = _silu(_B_ref(xn, B_w1, B_w2, B_w3, B_w4))
    return x + s * g
```

```python
import functools
import jax
import jax.numpy as jnp
import jax.experimental.pallas as pl
import jax.experimental.pallas.tpu as pltpu

F32 = jnp.float32
BF16 = jnp.bfloat16
EPS = 1e-5
HALO = 16
T_TILE = 256


def _ln(v):
    m = jnp.mean(v, axis=-1, keepdims=True)
    c = v - m
    var = jnp.mean(c * c, axis=-1, keepdims=True)
    return c * jax.lax.rsqrt(var + EPS)


def _gelu(v):
    c0 = 0.7978845608028654
    inner = v * (c0 + (c0 * 0.044715) * (v * v))
    return (0.5 * v) * (1.0 + jnp.tanh(inner))


def _nt(a, b):
    return jax.lax.dot_general(a, b, (((1,), (1,)), ((), ())), preferred_element_type=F32)


def _nn(a, b):
    return jnp.dot(a, b, preferred_element_type=F32)


def _kernel(x_ref, xnx_ref, xq_ref, lre_ref, lim_ref, ldt_ref, dsk_ref,
            bre_h, bim_h, cre_h, cim_h, w1_h, w2_h, w3_h, w4_h,
            o_ref,
            bre_s, bim_s, cre_s, cim_s, w1_s, w2_s, w3_s, w4_s, sems,
            ccat_s, tab_s, state_s, bu_s, hb_s, hh_s, xn_s, l2e_s, *, T, L, D):
    i = pl.program_id(0)
    srcs = (w1_h, bre_h, bim_h, w2_h, cre_h, cim_h, w3_h, w4_h)
    dsts = (w1_s, bre_s, bim_s, w2_s, cre_s, cim_s, w3_s, w4_s)

    def copy(k):
        return pltpu.make_async_copy(srcs[k], dsts[k], sems.at[k])

    def norm_rows(v):
        xn_ = _ln(v.astype(F32)).astype(BF16)
        l2_ = _ln(xn_.astype(F32)).astype(BF16)
        return xn_, l2_

    def init_tables():
        lre = lre_ref[...].reshape(1, D).astype(F32)
        lim = lim_ref[...].reshape(1, D).astype(F32)
        dt = jnp.exp(ldt_ref[...].reshape(1, D).astype(F32)).astype(BF16).astype(F32)
        zr = dt * lre
        zi = dt * lim
        row = jax.lax.broadcasted_iota(jnp.int32, (8, D), 0)
        for t, d in enumerate((1, 2, 4)):
            kk = float(d)
            ek = jnp.exp(kk * zr)
            pr = jnp.broadcast_to(ek * jnp.cos(kk * zi), (8, D))
            pi = jnp.broadcast_to(ek * jnp.sin(kk * zi), (8, D))
            tab_s[t, :, 0:D] = jnp.where(row >= d, pr, 0.0)
            tab_s[t, :, D:2 * D] = jnp.where(row >= d, pi, 0.0)
        kk = (row + 1).astype(F32)
        ek = jnp.exp(kk * zr)
        tab_s[3, :, 0:D] = ek * jnp.cos(kk * zi)
        tab_s[3, :, D:2 * D] = ek * jnp.sin(kk * zi)
        state_s[...] = jnp.zeros_like(state_s)

    def init_c():
        lre = lre_ref[...].reshape(1, D).astype(F32)
        lim = lim_ref[...].reshape(1, D).astype(F32)
        a_re = tab_s[3, 0:1, 0:D]
        a_im = tab_s[3, 0:1, D:2 * D]
        den = lre * lre + lim * lim
        nr = a_re - 1.0
        k_re = (nr * lre + a_im * lim) / den
        k_im = (a_im * lre - nr * lim) / den
        cre = cre_s[...].astype(F32)
        cim = cim_s[...].astype(F32)
        ccat_s[:, 0:D] = (2.0 * (cre * k_re - cim * k_im)).astype(BF16)
        ccat_s[:, D:2 * D] = (-2.0 * (cre * k_im + cim * k_re)).astype(BF16)

    def mixer_hidden(l2, row0):
        n = l2.shape[0]
        h = _gelu(_nn(l2, w1_s[...]))
        rows = jax.lax.broadcasted_iota(jnp.int32, (n, D), 0) + row0
        return jnp.where(rows < L, h, 0.0)

    def body(first, last):
        if first:
            copy(0).start()
            init_tables()
            copy(1).start()
            copy(2).start()
            xn_t, l2_t = norm_rows(x_ref[...])
            _, l2_n = norm_rows(xnx_ref[0:HALO, :])
            xn_s[...] = xn_t
            l2e_s[...] = jnp.concatenate([l2_t, l2_n], axis=0)
            copy(0).wait()
            hh_s[0:HALO, :] = jnp.zeros((HALO, D), F32)
            hh_s[HALO:, :] = mixer_hidden(l2e_s[...], 0)
            copy(1).wait()
            copy(2).wait()
            for k in range(3, 6):
                copy(k).start()

        xn_b = xn_s[...]
        bu_s[:, 0:D] = _nt(xn_b, bre_s[...])
        bu_s[:, D:2 * D] = _nt(xn_b, bim_s[...])

        c_re = state_s[:, 0:D]
        c_im = state_s[:, D:2 * D]
        prev = None
        for b in range(T // 8):
            hr = bu_s[b * 8:(b + 1) * 8, 0:D]
            hi = bu_s[b * 8:(b + 1) * 8, D:2 * D]
            for t, d in enumerate((1, 2, 4)):
                ar = tab_s[t, :, 0:D]
                ai = tab_s[t, :, D:2 * D]
                rr = pltpu.roll(hr, d, 0)
                ri = pltpu.roll(hi, d, 0)
                hr, hi = hr + ar * rr - ai * ri, hi + ar * ri + ai * rr
            pr = tab_s[3, :, 0:D]
            pi = tab_s[3, :, D:2 * D]
            hr, hi = hr + pr * c_re - pi * c_im, hi + pr * c_im + pi * c_re
            c_re = jnp.broadcast_to(hr[7:8, :], (8, D))
            c_im = jnp.broadcast_to(hi[7:8, :], (8, D))
            cur = jnp.concatenate([hr, hi], axis=1)
            if b % 2 == 0:
                prev = cur
            else:
                hb_s[(b - 1) * 8:(b + 1) * 8, :] = jnp.concatenate([prev, cur], axis=0).astype(BF16)
        state_s[:, 0:D] = c_re
        state_s[:, D:2 * D] = c_im

        if first:
            for k in range(3, 6):
                copy(k).wait()
            copy(6).start()
            init_c()

        xn = xn_b.astype(F32)

        c = D // 4
        lane = jax.lax.broadcasted_iota(jnp.int32, (T, D), 1)
        g0 = hh_s[pl.ds(HALO - 1, T), :]
        g1 = hh_s[pl.ds(HALO + 1, T), :]
        g2 = hh_s[pl.ds(HALO - 2, T), :]
        g3 = hh_s[pl.ds(HALO + 2, T), :]
        G = jnp.where(lane < c, g0, jnp.where(lane < 2 * c, g1, jnp.where(lane < 3 * c, g2, g3)))
        x1 = xn + _nn(G.astype(BF16), w2_s[...])
        l3 = _ln(x1).astype(BF16)
        ya = _nt(hb_s[:, 0:D], ccat_s[:, 0:D]) + xn * dsk_ref[...].reshape(1, D).astype(F32)

        if first:
            copy(6).wait()
            copy(7).start()

        u = _gelu(_nn(l3, w3_s[...])).astype(BF16)
        if first:
            copy(7).wait()
        z = x1 + _nn(u, w4_s[...])
        g = z * jax.nn.sigmoid(z)
        y = ya + _nt(hb_s[:, D:2 * D], ccat_s[:, D:2 * D])
        o_ref[...] = x_ref[...].astype(F32) + y * g

        if not last:
            xn_t, l2_t = norm_rows(xnx_ref[...])
            _, l2_n = norm_rows(xq_ref[...])
            xn_s[...] = xn_t
            l2w = jnp.concatenate([l2_t[HALO:, :], l2_n], axis=0)
            hh_s[0:2 * HALO, :] = hh_s[T:T + 2 * HALO, :]
            hh_s[2 * HALO:, :] = mixer_hidden(l2w, (i + 1) * T + HALO)

    nt = pl.num_programs(0)

    @pl.when(i == 0)
    def _():
        body(True, False)

    @pl.when((i > 0) & (i < nt - 1))
    def _():
        body(False, False)

    @pl.when(i == nt - 1)
    def _():
        body(False, True)


@jax.jit
def pallas_recurrent_scan__ssm_conv_s5__mixer_s_mlp__prompt_kernel(
    A_x, A_Lambda_re, A_Lambda_im, A_B_re, A_B_im, A_C_re, A_C_im, A_log_dt, A_Dskip,
    B_x, B_w1, B_w2, B_w3, B_w4,
):
    Bsz, L, D = A_x.shape
    assert Bsz == 1
    P = A_Lambda_re.shape[0]
    F = B_w3.shape[1]
    T = T_TILE
    nt = L // T
    x2 = A_x.reshape(L, D)
    hb = T // HALO
    nhb = L // HALO
    vec = lambda n: pl.BlockSpec((n,), lambda i: (0,))
    anyspec = pl.BlockSpec(memory_space=pl.ANY)
    in_specs = [
        pl.BlockSpec((T, D), lambda i: (i, 0)),
        pl.BlockSpec((T, D), lambda i: (jnp.minimum(i + 1, nt - 1), 0)),
        pl.BlockSpec((HALO, D), lambda i: (jnp.minimum((i + 2) * hb, nhb - 1), 0)),
        vec(P), vec(P), vec(P), vec(D),
    ] + [anyspec] * 8
    out = pl.pallas_call(
        functools.partial(_kernel, T=T, L=L, D=D),
        grid=(nt,),
        in_specs=in_specs,
        out_specs=pl.BlockSpec((T, D), lambda i: (i, 0)),
        out_shape=jax.ShapeDtypeStruct((L, D), F32),
        scratch_shapes=[
            pltpu.VMEM((P, D), BF16), pltpu.VMEM((P, D), BF16),
            pltpu.VMEM((D, P), BF16), pltpu.VMEM((D, P), BF16),
            pltpu.VMEM((D, D), BF16), pltpu.VMEM((D, D), BF16),
            pltpu.VMEM((D, F), BF16), pltpu.VMEM((F, D), BF16),
            pltpu.SemaphoreType.DMA((8,)),
            pltpu.VMEM((D, 2 * P), BF16),
            pltpu.VMEM((4, 8, 2 * P), F32),
            pltpu.VMEM((8, 2 * P), F32),
            pltpu.VMEM((T, 2 * P), F32),
            pltpu.VMEM((T, 2 * P), BF16),
            pltpu.VMEM((T + 2 * HALO, D), F32),
            pltpu.VMEM((T, D), BF16),
            pltpu.VMEM((T + HALO, D), BF16),
        ],
        compiler_params=pltpu.CompilerParams(
            dimension_semantics=("arbitrary",),
            vmem_limit_bytes=100 * 1024 * 1024,
        ),
    )(x2, x2, x2, A_Lambda_re, A_Lambda_im, A_log_dt, A_Dskip,
      A_B_re, A_B_im, A_C_re, A_C_im, B_w1, B_w2, B_w3, B_w4)
    return out.reshape(Bsz, L, D)
```

```python
import functools

import jax
import jax.numpy as jnp
import jax.experimental.pallas as pl
import jax.experimental.pallas.tpu as pltpu

F32 = jnp.float32
BF16 = jnp.bfloat16
EPS = 1e-5
HALO = 16
T_TILE = 256


def _ln(v):
    m = jnp.mean(v, axis=-1, keepdims=True)
    c = v - m
    var = jnp.mean(c * c, axis=-1, keepdims=True)
    return c * jax.lax.rsqrt(var + EPS)


def _gelu(v):
    c0 = 0.7978845608028654
    inner = v * (c0 + (c0 * 0.044715) * (v * v))
    return (0.5 * v) * (1.0 + jnp.tanh(inner))


def _nt(a, b):
    return jax.lax.dot_general(a, b, (((1,), (1,)), ((), ())), preferred_element_type=F32)


def _nn(a, b):
    return jnp.dot(a, b, preferred_element_type=F32)


def _kernel(x_ref, xnx_ref, xq_ref, lre_ref, lim_ref, ldt_ref, dsk_ref,
            bre_h, bim_h, cre_h, cim_h, w1_h, w2_h, w3_h, w4_h,
            o_ref,
            bre_s, bim_s, cre_s, cim_s, w1_s, w2_s, w3_s, w4_s, sems,
            ccat_s, tab_s, state_s, bu_s, hb_s, hh_s, xn_s, l2e_s, *, T, L, D):
    i = pl.program_id(0)
    NCT = D // 128
    srcs = (w1_h, bre_h, bim_h, w2_h, cre_h, cim_h, w3_h, w4_h)
    dsts = (w1_s, bre_s, bim_s, w2_s, cre_s, cim_s, w3_s, w4_s)

    def copy(k):
        return pltpu.make_async_copy(srcs[k], dsts[k], sems.at[k])

    def norm_rows(v):
        xn_ = _ln(v.astype(F32)).astype(BF16)
        l2_ = _ln(xn_.astype(F32)).astype(BF16)
        return xn_, l2_

    def init_tables():
        lre = lre_ref[...].reshape(1, D).astype(F32)
        lim = lim_ref[...].reshape(1, D).astype(F32)
        dt = jnp.exp(ldt_ref[...].reshape(1, D).astype(F32)).astype(BF16).astype(F32)
        zr = dt * lre
        zi = dt * lim
        row = jax.lax.broadcasted_iota(jnp.int32, (8, D), 0)
        for t, d in enumerate((1, 2, 4)):
            kk = float(d)
            ek = jnp.exp(kk * zr)
            pr = jnp.broadcast_to(ek * jnp.cos(kk * zi), (8, D))
            pi = jnp.broadcast_to(ek * jnp.sin(kk * zi), (8, D))
            tab_s[t, :, 0:D] = jnp.where(row >= d, pr, 0.0)
            tab_s[t, :, D:2 * D] = jnp.where(row >= d, pi, 0.0)
        kk = (row + 1).astype(F32)
        ek = jnp.exp(kk * zr)
        tab_s[3, :, 0:D] = ek * jnp.cos(kk * zi)
        tab_s[3, :, D:2 * D] = ek * jnp.sin(kk * zi)
        state_s[...] = jnp.zeros_like(state_s)

    def init_c():
        lre = lre_ref[...].reshape(1, D).astype(F32)
        lim = lim_ref[...].reshape(1, D).astype(F32)
        a_re = tab_s[3, 0:1, 0:D]
        a_im = tab_s[3, 0:1, D:2 * D]
        den = lre * lre + lim * lim
        nr = a_re - 1.0
        k_re = (nr * lre + a_im * lim) / den
        k_im = (a_im * lre - nr * lim) / den
        cre = cre_s[...].astype(F32)
        cim = cim_s[...].astype(F32)
        ccat_s[:, 0:D] = (2.0 * (cre * k_re - cim * k_im)).astype(BF16)
        ccat_s[:, D:2 * D] = (-2.0 * (cre * k_im + cim * k_re)).astype(BF16)

    def mixer_hidden(l2, row0):
        n = l2.shape[0]
        h = _gelu(_nn(l2, w1_s[...]))
        rows = jax.lax.broadcasted_iota(jnp.int32, (n, D), 0) + row0
        return jnp.where(rows < L, h, 0.0)

    def next_front():
        xn_t, l2_t = norm_rows(xnx_ref[...])
        _, l2_n = norm_rows(xq_ref[...])
        xn_s[...] = xn_t
        l2w = jnp.concatenate([l2_t[HALO:, :], l2_n], axis=0)
        hh_s[0:2 * HALO, :] = hh_s[T:T + 2 * HALO, :]
        hh_s[2 * HALO:, :] = mixer_hidden(l2w, (i + 1) * T + HALO)

    def body(first, last):
        if first:
            copy(0).start()
            init_tables()
            copy(1).start()
            copy(2).start()
            xn_t, l2_t = norm_rows(x_ref[...])
            _, l2_n = norm_rows(xnx_ref[0:HALO, :])
            xn_s[...] = xn_t
            l2e_s[...] = jnp.concatenate([l2_t, l2_n], axis=0)
            copy(0).wait()
            copy(3).start()
            copy(4).start()
            copy(5).start()
            hh_s[0:HALO, :] = jnp.zeros((HALO, D), F32)
            hh_s[HALO:, :] = mixer_hidden(l2e_s[...], 0)
            copy(1).wait()
            copy(2).wait()
            copy(6).start()

        xn_b = xn_s[...]
        for cc in range(NCT):
            lo, hi_ = cc * 128, (cc + 1) * 128
            bu_s[:, lo:hi_] = _nt(xn_b, bre_s[lo:hi_, :])
            bu_s[:, D + lo:D + hi_] = _nt(xn_b, bim_s[lo:hi_, :])

        c_re = state_s[:, 0:D]
        c_im = state_s[:, D:2 * D]
        prev = None
        for b in range(T // 8):
            hr = bu_s[b * 8:(b + 1) * 8, 0:D]
            hi = bu_s[b * 8:(b + 1) * 8, D:2 * D]
            for t, d in enumerate((1, 2, 4)):
                ar = tab_s[t, :, 0:D]
                ai = tab_s[t, :, D:2 * D]
                rr = pltpu.roll(hr, d, 0)
                ri = pltpu.roll(hi, d, 0)
                hr, hi = hr + ar * rr - ai * ri, hi + ar * ri + ai * rr
            pr = tab_s[3, :, 0:D]
            pi = tab_s[3, :, D:2 * D]
            hr, hi = hr + pr * c_re - pi * c_im, hi + pr * c_im + pi * c_re
            c_re = jnp.broadcast_to(hr[7:8, :], (8, D))
            c_im = jnp.broadcast_to(hi[7:8, :], (8, D))
            cur = jnp.concatenate([hr, hi], axis=1)
            if b % 2 == 0:
                prev = cur
            else:
                hb_s[(b - 1) * 8:(b + 1) * 8, :] = jnp.concatenate([prev, cur], axis=0).astype(BF16)
        state_s[:, 0:D] = c_re
        state_s[:, D:2 * D] = c_im

        if first:
            for k in range(3, 6):
                copy(k).wait()
            copy(7).start()
            init_c()

        xn = xn_b.astype(F32)

        c = D // 4
        lane = jax.lax.broadcasted_iota(jnp.int32, (T, D), 1)
        g0 = hh_s[pl.ds(HALO - 1, T), :]
        g1 = hh_s[pl.ds(HALO + 1, T), :]
        g2 = hh_s[pl.ds(HALO - 2, T), :]
        g3 = hh_s[pl.ds(HALO + 2, T), :]
        G = jnp.where(lane < c, g0, jnp.where(lane < 2 * c, g1, jnp.where(lane < 3 * c, g2, g3)))
        Gb = G.astype(BF16)
        x1 = xn
        for cc in range(NCT):
            lo, hi_ = cc * 128, (cc + 1) * 128
            x1 = x1 + _nn(Gb[:, lo:hi_], w2_s[lo:hi_, :])
        l3 = _ln(x1).astype(BF16)
        ya = _nt(hb_s[:, 0:D], ccat_s[:, 0:D]) + xn * dsk_ref[...].reshape(1, D).astype(F32)

        if first:
            next_front()
            copy(6).wait()

        u = _gelu(_nn(l3, w3_s[...])).astype(BF16)
        if first:
            copy(7).wait()
        z = x1 + _nn(u, w4_s[...])
        g = z * jax.nn.sigmoid(z)
        if not last and not first:
            next_front()
        y = ya + _nt(hb_s[:, D:2 * D], ccat_s[:, D:2 * D])
        o_ref[...] = x_ref[...].astype(F32) + y * g

    nt = pl.num_programs(0)

    @pl.when(i == 0)
    def _():
        body(True, False)

    @pl.when((i > 0) & (i < nt - 1))
    def _():
        body(False, False)

    @pl.when(i == nt - 1)
    def _():
        body(False, True)


@jax.jit
def pallas_recurrent_scan__ssm_conv_s5__mixer_s_mlp__prompt_kernel(
    A_x: jax.Array,
    A_Lambda_re: jax.Array,
    A_Lambda_im: jax.Array,
    A_B_re: jax.Array,
    A_B_im: jax.Array,
    A_C_re: jax.Array,
    A_C_im: jax.Array,
    A_log_dt: jax.Array,
    A_Dskip: jax.Array,
    B_x: jax.Array,
    B_w1: jax.Array,
    B_w2: jax.Array,
    B_w3: jax.Array,
    B_w4: jax.Array,
):
    Bsz, L, D = A_x.shape
    P = A_Lambda_re.shape[0]
    F = B_w3.shape[1]
    T = T_TILE
    assert Bsz == 1 and P == D and L % T == 0 and L // T >= 3 and D % 128 == 0
    nt = L // T
    x2 = A_x.reshape(L, D)
    hb = T // HALO
    nhb = L // HALO
    vec = lambda n: pl.BlockSpec((n,), lambda i: (0,))
    anyspec = pl.BlockSpec(memory_space=pl.ANY)
    in_specs = [
        pl.BlockSpec((T, D), lambda i: (i, 0)),
        pl.BlockSpec((T, D), lambda i: (jnp.minimum(i + 1, nt - 1), 0)),
        pl.BlockSpec((HALO, D), lambda i: (jnp.minimum((i + 2) * hb, nhb - 1), 0)),
        vec(P), vec(P), vec(P), vec(D),
    ] + [anyspec] * 8
    out = pl.pallas_call(
        functools.partial(_kernel, T=T, L=L, D=D),
        grid=(nt,),
        in_specs=in_specs,
        out_specs=pl.BlockSpec((T, D), lambda i: (i, 0)),
        out_shape=jax.ShapeDtypeStruct((L, D), F32),
        scratch_shapes=[
            pltpu.VMEM((P, D), BF16), pltpu.VMEM((P, D), BF16),
            pltpu.VMEM((D, P), BF16), pltpu.VMEM((D, P), BF16),
            pltpu.VMEM((D, D), BF16), pltpu.VMEM((D, D), BF16),
            pltpu.VMEM((D, F), BF16), pltpu.VMEM((F, D), BF16),
            pltpu.SemaphoreType.DMA((8,)),
            pltpu.VMEM((D, 2 * P), BF16),
            pltpu.VMEM((4, 8, 2 * P), F32),
            pltpu.VMEM((8, 2 * P), F32),
            pltpu.VMEM((T, 2 * P), F32),
            pltpu.VMEM((T, 2 * P), BF16),
            pltpu.VMEM((T + 2 * HALO, D), F32),
            pltpu.VMEM((T, D), BF16),
            pltpu.VMEM((T + HALO, D), BF16),
        ],
        compiler_params=pltpu.CompilerParams(
            dimension_semantics=("arbitrary",),
            vmem_limit_bytes=100 * 1024 * 1024,
        ),
    )(x2, x2, x2, A_Lambda_re, A_Lambda_im, A_log_dt, A_Dskip,
      A_B_re, A_B_im, A_C_re, A_C_im, B_w1, B_w2, B_w3, B_w4)
    return out.reshape(Bsz, L, D)
```

```python
import functools

import jax
import jax.numpy as jnp
import jax.experimental.pallas as pl
import jax.experimental.pallas.tpu as pltpu

F32 = jnp.float32
BF16 = jnp.bfloat16
EPS = 1e-5
HALO = 16
T_TILE = 256


def _ln(v):
    m = jnp.mean(v, axis=-1, keepdims=True)
    c = v - m
    var = jnp.mean(c * c, axis=-1, keepdims=True)
    return c * jax.lax.rsqrt(var + EPS)


def _gelu(v):
    c0 = 0.7978845608028654
    inner = v * (c0 + (c0 * 0.044715) * (v * v))
    return (0.5 * v) * (1.0 + jnp.tanh(inner))


def _nt(a, b):
    return jax.lax.dot_general(a, b, (((1,), (1,)), ((), ())), preferred_element_type=F32)


def _nn(a, b):
    return jnp.dot(a, b, preferred_element_type=F32)


def _kernel(x_ref, xnx_ref, xq_ref, lre_ref, lim_ref, ldt_ref, dsk_ref,
            bre_h, bim_h, cre_h, cim_h, w1_h, w2_h, w3_h, w4_h,
            o_ref,
            bre_s, bim_s, cre_s, cim_s, w1_s, w2_s, w3_s, w4_s, sems,
            ccat_s, tab_s, state_s, bu_s, hb_s, hh_s, xn_s, l2e_s, *, T, L, D):
    i = pl.program_id(0)
    NCT = D // 128
    srcs = (w1_h, bre_h, bim_h, w2_h, cre_h, cim_h, w3_h, w4_h)
    dsts = (w1_s, bre_s, bim_s, w2_s, cre_s, cim_s, w3_s, w4_s)

    def copy(k):
        return pltpu.make_async_copy(srcs[k], dsts[k], sems.at[k])

    def norm_rows(v):
        xn_ = _ln(v.astype(F32)).astype(BF16)
        l2_ = _ln(xn_.astype(F32)).astype(BF16)
        return xn_, l2_

    def init_tables():
        lre = lre_ref[...].reshape(1, D).astype(F32)
        lim = lim_ref[...].reshape(1, D).astype(F32)
        dt = jnp.exp(ldt_ref[...].reshape(1, D).astype(F32)).astype(BF16).astype(F32)
        zr = dt * lre
        zi = dt * lim
        row = jax.lax.broadcasted_iota(jnp.int32, (8, D), 0)
        for t, d in enumerate((1, 2, 4)):
            kk = float(d)
            ek = jnp.exp(kk * zr)
            pr = jnp.broadcast_to(ek * jnp.cos(kk * zi), (8, D))
            pi = jnp.broadcast_to(ek * jnp.sin(kk * zi), (8, D))
            tab_s[t, :, 0:D] = jnp.where(row >= d, pr, 0.0)
            tab_s[t, :, D:2 * D] = jnp.where(row >= d, pi, 0.0)
        kk = (row + 1).astype(F32)
        ek = jnp.exp(kk * zr)
        tab_s[3, :, 0:D] = ek * jnp.cos(kk * zi)
        tab_s[3, :, D:2 * D] = ek * jnp.sin(kk * zi)
        state_s[...] = jnp.zeros_like(state_s)

    def init_c():
        lre = lre_ref[...].reshape(1, D).astype(F32)
        lim = lim_ref[...].reshape(1, D).astype(F32)
        a_re = tab_s[3, 0:1, 0:D]
        a_im = tab_s[3, 0:1, D:2 * D]
        den = lre * lre + lim * lim
        nr = a_re - 1.0
        k_re = (nr * lre + a_im * lim) / den
        k_im = (a_im * lre - nr * lim) / den
        cre = cre_s[...].astype(F32)
        cim = cim_s[...].astype(F32)
        ccat_s[:, 0:D] = (2.0 * (cre * k_re - cim * k_im)).astype(BF16)
        ccat_s[:, D:2 * D] = (-2.0 * (cre * k_im + cim * k_re)).astype(BF16)

    def mixer_hidden(l2, row0):
        n = l2.shape[0]
        h = _gelu(_nn(l2, w1_s[...]))
        rows = jax.lax.broadcasted_iota(jnp.int32, (n, D), 0) + row0
        return jnp.where(rows < L, h, 0.0)

    def next_front():
        xn_t, l2_t = norm_rows(xnx_ref[...])
        _, l2_n = norm_rows(xq_ref[...])
        xn_s[...] = xn_t
        l2w = jnp.concatenate([l2_t[HALO:, :], l2_n], axis=0)
        hh_s[0:2 * HALO, :] = hh_s[T:T + 2 * HALO, :]
        hh_s[2 * HALO:, :] = mixer_hidden(l2w, (i + 1) * T + HALO)

    def body(first, last):
        if first:
            copy(0).start()
            init_tables()
            copy(1).start()
            copy(2).start()
            xn_t, l2_t = norm_rows(x_ref[...])
            _, l2_n = norm_rows(xnx_ref[0:HALO, :])
            xn_s[...] = xn_t
            l2e_s[...] = jnp.concatenate([l2_t, l2_n], axis=0)
            copy(0).wait()
            copy(3).start()
            copy(4).start()
            copy(5).start()
            hh_s[0:HALO, :] = jnp.zeros((HALO, D), F32)
            hh_s[HALO:, :] = mixer_hidden(l2e_s[...], 0)
            copy(1).wait()
            copy(2).wait()
            copy(6).start()

        xn_b = xn_s[...]
        for cc in range(NCT):
            lo, hi_ = cc * 128, (cc + 1) * 128
            bu_s[:, lo:hi_] = _nt(xn_b, bre_s[lo:hi_, :])
            bu_s[:, D + lo:D + hi_] = _nt(xn_b, bim_s[lo:hi_, :])

        c_re = state_s[:, 0:D]
        c_im = state_s[:, D:2 * D]
        prev = None
        for b in range(T // 8):
            hr = bu_s[b * 8:(b + 1) * 8, 0:D]
            hi = bu_s[b * 8:(b + 1) * 8, D:2 * D]
            for t, d in enumerate((1, 2, 4)):
                ar = tab_s[t, :, 0:D]
                ai = tab_s[t, :, D:2 * D]
                rr = pltpu.roll(hr, d, 0)
                ri = pltpu.roll(hi, d, 0)
                hr, hi = hr + ar * rr - ai * ri, hi + ar * ri + ai * rr
            pr = tab_s[3, :, 0:D]
            pi = tab_s[3, :, D:2 * D]
            hr, hi = hr + pr * c_re - pi * c_im, hi + pr * c_im + pi * c_re
            c_re = jnp.broadcast_to(hr[7:8, :], (8, D))
            c_im = jnp.broadcast_to(hi[7:8, :], (8, D))
            cur = jnp.concatenate([hr, hi], axis=1)
            if b % 2 == 0:
                prev = cur
            else:
                hb_s[(b - 1) * 8:(b + 1) * 8, :] = jnp.concatenate([prev, cur], axis=0).astype(BF16)
        state_s[:, 0:D] = c_re
        state_s[:, D:2 * D] = c_im

        if first:
            for k in range(3, 6):
                copy(k).wait()
            copy(7).start()
            init_c()

        xn = xn_b.astype(F32)

        q = D // 4
        shifts = (-1, 1, -2, 2)
        lane = jax.lax.broadcasted_iota(jnp.int32, (T, 128), 1)
        x1 = xn
        for cc in range(NCT):
            lo, hi_ = cc * 128, (cc + 1) * 128
            grp = sorted({min(l // q, 3) for l in range(lo, hi_)})
            gt = hh_s[pl.ds(HALO + shifts[grp[-1]], T), lo:hi_]
            for gidx in reversed(grp[:-1]):
                gt = jnp.where(lane < (gidx + 1) * q - lo,
                               hh_s[pl.ds(HALO + shifts[gidx], T), lo:hi_], gt)
            x1 = x1 + _nn(gt.astype(BF16), w2_s[lo:hi_, :])
        l3 = _ln(x1).astype(BF16)
        ya = _nt(hb_s[:, 0:D], ccat_s[:, 0:D]) + xn * dsk_ref[...].reshape(1, D).astype(F32)

        if first:
            next_front()
            copy(6).wait()

        u = _gelu(_nn(l3, w3_s[...])).astype(BF16)
        if first:
            copy(7).wait()
        z = x1 + _nn(u, w4_s[...])
        g = z * jax.nn.sigmoid(z)
        if not last and not first:
            next_front()
        y = ya + _nt(hb_s[:, D:2 * D], ccat_s[:, D:2 * D])
        o_ref[...] = x_ref[...].astype(F32) + y * g

    nt = pl.num_programs(0)

    @pl.when(i == 0)
    def _():
        body(True, False)

    @pl.when((i > 0) & (i < nt - 1))
    def _():
        body(False, False)

    @pl.when(i == nt - 1)
    def _():
        body(False, True)


@jax.jit
def pallas_recurrent_scan__ssm_conv_s5__mixer_s_mlp__prompt_kernel(
    A_x: jax.Array,
    A_Lambda_re: jax.Array,
    A_Lambda_im: jax.Array,
    A_B_re: jax.Array,
    A_B_im: jax.Array,
    A_C_re: jax.Array,
    A_C_im: jax.Array,
    A_log_dt: jax.Array,
    A_Dskip: jax.Array,
    B_x: jax.Array,
    B_w1: jax.Array,
    B_w2: jax.Array,
    B_w3: jax.Array,
    B_w4: jax.Array,
):
    Bsz, L, D = A_x.shape
    P = A_Lambda_re.shape[0]
    F = B_w3.shape[1]
    T = T_TILE
    assert Bsz == 1 and P == D and L % T == 0 and L // T >= 3 and D % 128 == 0
    nt = L // T
    x2 = A_x.reshape(L, D)
    hb = T // HALO
    nhb = L // HALO
    vec = lambda n: pl.BlockSpec((n,), lambda i: (0,))
    anyspec = pl.BlockSpec(memory_space=pl.ANY)
    in_specs = [
        pl.BlockSpec((T, D), lambda i: (i, 0)),
        pl.BlockSpec((T, D), lambda i: (jnp.minimum(i + 1, nt - 1), 0)),
        pl.BlockSpec((HALO, D), lambda i: (jnp.minimum((i + 2) * hb, nhb - 1), 0)),
        vec(P), vec(P), vec(P), vec(D),
    ] + [anyspec] * 8
    out = pl.pallas_call(
        functools.partial(_kernel, T=T, L=L, D=D),
        grid=(nt,),
        in_specs=in_specs,
        out_specs=pl.BlockSpec((T, D), lambda i: (i, 0)),
        out_shape=jax.ShapeDtypeStruct((L, D), F32),
        scratch_shapes=[
            pltpu.VMEM((P, D), BF16), pltpu.VMEM((P, D), BF16),
            pltpu.VMEM((D, P), BF16), pltpu.VMEM((D, P), BF16),
            pltpu.VMEM((D, D), BF16), pltpu.VMEM((D, D), BF16),
            pltpu.VMEM((D, F), BF16), pltpu.VMEM((F, D), BF16),
            pltpu.SemaphoreType.DMA((8,)),
            pltpu.VMEM((D, 2 * P), BF16),
            pltpu.VMEM((4, 8, 2 * P), F32),
            pltpu.VMEM((8, 2 * P), F32),
            pltpu.VMEM((T, 2 * P), F32),
            pltpu.VMEM((T, 2 * P), BF16),
            pltpu.VMEM((T + 2 * HALO, D), F32),
            pltpu.VMEM((T, D), BF16),
            pltpu.VMEM((T + HALO, D), BF16),
        ],
        compiler_params=pltpu.CompilerParams(
            dimension_semantics=("arbitrary",),
            vmem_limit_bytes=100 * 1024 * 1024,
        ),
    )(x2, x2, x2, A_Lambda_re, A_Lambda_im, A_log_dt, A_Dskip,
      A_B_re, A_B_im, A_C_re, A_C_im, B_w1, B_w2, B_w3, B_w4)
    return out.reshape(Bsz, L, D)
```
